```python
import os as _os
_os.environ.setdefault('JAX_PLATFORMS', 'cpu')
import jax
import jax.numpy as jnp

def _softmax(x, axis=-1):
    return jax.nn.softmax(x, axis=axis)

def _gelu(x):
    return jax.nn.gelu(x, approximate=True)

def _silu(x):
    return jax.nn.silu(x)

def _sigmoid(x):
    return jax.nn.sigmoid(x)

def _layernorm(x, axis=-1, eps=1e-05):
    m = jnp.mean(x, axis=axis, keepdims=True)
    v = jnp.var(x, axis=axis, keepdims=True)
    return (x - m) / jnp.sqrt(v + eps)

def _scatter_add(tgt, idx, src, axis=0):
    return tgt.at[idx].add(src)

def _segment_sum(src, seg, n):
    return jax.ops.segment_sum(src, seg, n)

class _Rng:

    def __init__(self, key):
        self._k = key

    def _next(self):
        self._k, sub = jax.random.split(self._k)
        return sub

    def normal(self, shape):
        return jax.random.normal(self._next(), shape, dtype=jnp.bfloat16)

    def randint(self, lo, hi, shape):
        return jax.random.randint(self._next(), shape, lo, hi, dtype=jnp.int32)

    def uniform(self, shape, lo=0.0, hi=1.0):
        return jax.random.uniform(self._next(), shape, jnp.bfloat16, lo, hi)

    def permutation(self, n):
        return jax.random.permutation(self._next(), n)
kernel_name = 'gated_mix__memory_aug_recurrent_mem_tr__glu_gated_geglu__prompt'

def setup_inputs():
    _rng = _Rng(jax.random.key(int.from_bytes(__import__("os").urandom(4), "little")))
    _w = lambda a: (lambda t: t.astype(jnp.bfloat16) if jnp.issubdtype(t.dtype, jnp.floating) else t)(jnp.asarray(a))

    def _A_setup():
        B, S, Dm = (1, 2048, 640)
        H, Dh = (32, 128)
        M, seg = (8, 32)
        seg = min(seg, S)
        S = S // seg * seg
        return {'x': _w((lambda *s: _rng.normal(s) * 0.05)(B, S, Dm)), 'mem0': _w((lambda *s: _rng.normal(s) * 0.4)(B, M, Dm)), 'Wq': _w((lambda *s: _rng.normal(s) * 3.2)(Dm, H, Dh) * Dm ** (-0.5)), 'Wk': _w((lambda *s: _rng.normal(s) * 3.2)(Dm, H, Dh) * Dm ** (-0.5)), 'Wv': _w((lambda *s: _rng.normal(s) * 0.4)(Dm, H, Dh) * Dm ** (-0.5)), 'Wo': _w((lambda *s: _rng.normal(s) * 0.4)(H, Dh, Dm) * (H * Dh) ** (-0.5)), 'seg_len': seg}
    _A_in = _A_setup()

    def _B_setup():
        B, S, Dm, Df = (1, 2048, 640, 1728)
        return {'x': _w((lambda *s: _rng.normal(s) * 0.05)(B, S, Dm)), 'w_gate': _w((lambda *s: _rng.normal(s) * 1.6)(Dm, Df) * Dm ** (-0.5)), 'w_up': _w((lambda *s: _rng.normal(s) * 1.6)(Dm, Df) * Dm ** (-0.5)), 'w_down': _w((lambda *s: _rng.normal(s) * 1.6)(Df, Dm) * Df ** (-0.5))}
    _B_in = _B_setup()
    return {'A_x': _A_in['x'], 'A_mem0': _A_in['mem0'], 'A_Wq': _A_in['Wq'], 'A_Wk': _A_in['Wk'], 'A_Wv': _A_in['Wv'], 'A_Wo': _A_in['Wo'], 'A_seg_len': _A_in['seg_len'], 'B_x': _B_in['x'], 'B_w_gate': _B_in['w_gate'], 'B_w_up': _B_in['w_up'], 'B_w_down': _B_in['w_down'], 'gate_w': _w((lambda *s: _rng.normal(s) * 0.05)(640) * 16.0)}

def reference(A_x, A_mem0, A_Wq, A_Wk, A_Wv, A_Wo, A_seg_len, B_x, B_w_gate, B_w_up, B_w_down, gate_w):

    def _A_ref(x, mem0, Wq, Wk, Wv, Wo, seg_len):
        B, S, Dm = x.shape
        H, Dh = (Wq.shape[1], Wq.shape[2])
        M = mem0.shape[1]
        scale = Dh ** (-0.5)
        n_seg = S // seg_len
        L = M + seg_len
        idx = jnp.arange(L)
        mask = (idx[:, None] < M) | (idx[:, None] >= idx[None, :])
        mem = mem0
        outs = []
        for s in range(n_seg):
            xs = x[:, s * seg_len:(s + 1) * seg_len, :].copy()
            h = jnp.concatenate([mem, xs], axis=1)
            q = jnp.einsum('btd,dhe->bhte', h, Wq)
            k = jnp.einsum('btd,dhe->bhte', h, Wk)
            v = jnp.einsum('btd,dhe->bhte', h, Wv)
            scores = jnp.einsum('bhqe,bhke->bhqk', q, k) * scale
            scores = jnp.where(mask[None, None], scores, -1000000000.0)
            p = _softmax(scores, axis=-1)
            o = jnp.einsum('bhqk,bhke->bhqe', p, v)
            o = jnp.einsum('bhte,hed->btd', o, Wo)
            mem = o[:, :M, :].copy()
            outs.append(o[:, M:, :])
        return jnp.concatenate(outs, axis=1)

    def _B_ref(x, w_gate, w_up, w_down):
        g = jnp.einsum('bsd,df->bsf', x, w_gate)
        u = jnp.einsum('bsd,df->bsf', x, w_up)
        h = _gelu(g) * u
        return jnp.einsum('bsf,fd->bsd', h, w_down)
    x = A_x
    g = _sigmoid((x * gate_w).sum(-1, keepdims=True))
    a = _A_ref(x, A_mem0, A_Wq, A_Wk, A_Wv, A_Wo, A_seg_len)
    b = _B_ref(x, B_w_gate, B_w_up, B_w_down)
    return g * a + (1 - g) * b
```

```python
import jax
import jax.numpy as jnp
from jax import lax
import jax.experimental.pallas as pl
import jax.experimental.pallas.tpu as pltpu

S, D, H, E, M, SEG, DF = 2048, 640, 32, 128, 8, 32, 1728
HE = H * E
NS = S // SEG
R = 48
G = 4
BF, F32 = jnp.bfloat16, jnp.float32
NT = (((1,), (1,)), ((), ()))


def _dot(a, b):
    return jnp.dot(a, b, preferred_element_type=F32)


def _kernel(x_h, mem_ref, gw_ref, wq_h, wk_h, wv_h, wo_h, wg_h, wu_h, wd_h, out_ref,
            x, wq, wk, wv, wo, wg, wu, wd, acc, gate, sem):
    srcs = (x_h, wg_h, wu_h, wd_h, wk_h, wv_h, wq_h, wo_h)
    dsts = (x, wg, wu, wd, wk, wv, wq, wo)
    cps = [pltpu.make_async_copy(s, d, sem.at[i]) for i, (s, d) in enumerate(zip(srcs, dsts))]
    for c in cps:
        c.start()
    for c in cps[:4]:
        c.wait()
    scale = E ** -0.5
    TM = 256

    def ffn(i, _):
        r = pl.ds(pl.multiple_of(i * TM, TM), TM)
        xs = x[r, :]
        g = jax.nn.sigmoid(jnp.sum(xs.astype(F32) * gw_ref[...].astype(F32), -1, keepdims=True))
        hh = jax.nn.gelu(_dot(xs, wg[...]), approximate=True) * _dot(xs, wu[...])
        acc[r, :] = (1.0 - g) * _dot(hh.astype(BF), wd[...])
        gate[r, :] = jnp.broadcast_to(g, (TM, 128))
        return 0
    lax.fori_loop(0, S // TM, ffn, 0)
    cps[4].wait()
    cps[5].wait()

    cps[6].wait()
    cps[7].wait()

    ri = lax.broadcasted_iota(jnp.int32, (R, R), 0)
    ci = lax.broadcasted_iota(jnp.int32, (R, R), 1)
    ok = (ci < SEG + M) & ((ci >= SEG) | (ri >= SEG) | (ci <= ri))
    zpad = jnp.zeros((8, D), F32)

    def chain(s, mem):
        r = pl.ds(pl.multiple_of(s * SEG, SEG), SEG)
        hh = jnp.concatenate([x[r, :], jnp.concatenate([mem, zpad], 0).astype(BF)], 0)
        q = _dot(hh, wq[...]).astype(BF)
        k = _dot(hh, wk[...]).astype(BF)
        v = _dot(hh, wv[...]).astype(BF)
        os_ = []
        for h in range(H):
            c = slice(h * E, (h + 1) * E)
            sc = lax.dot_general(q[:, c], k[:, c], NT, preferred_element_type=F32) * scale
            sc = jnp.where(ok, sc, -1e9)
            p = jnp.exp(sc - jnp.max(sc, -1, keepdims=True))
            p = p * (1.0 / jnp.sum(p, -1, keepdims=True))
            os_.append(_dot(p.astype(BF), v[:, c]).astype(BF))
        a = _dot(jnp.concatenate(os_, 1), wo[...])
        out_ref[r, :] = (gate[r, :][:, :1] * a[:SEG] + acc[r, :]).astype(out_ref.dtype)
        return a[SEG:SEG + M]
    lax.fori_loop(0, NS, chain, mem_ref[...].astype(F32))


@jax.jit
def pallas_gated_mix__memory_aug_recurrent_mem_tr__glu_gated_geglu__prompt_kernel(
    A_x, A_mem0, A_Wq, A_Wk, A_Wv, A_Wo, A_seg_len, B_x, B_w_gate, B_w_up, B_w_down, gate_w,
):
    anys = pl.BlockSpec(memory_space=pl.ANY)
    vm = pl.BlockSpec(memory_space=pltpu.VMEM)
    V = pltpu.VMEM
    out = pl.pallas_call(
        _kernel,
        out_shape=jax.ShapeDtypeStruct((S, D), A_x.dtype),
        in_specs=[anys, vm, vm] + [anys] * 7,
        out_specs=vm,
        scratch_shapes=[V((S, D), BF), V((D, HE), BF), V((D, HE), BF), V((D, HE), BF), V((HE, D), BF),
                        V((D, DF), BF), V((D, DF), BF), V((DF, D), BF),
                        V((S, D), F32), V((S, 128), F32),
                        pltpu.SemaphoreType.DMA((8,))],
        compiler_params=pltpu.CompilerParams(vmem_limit_bytes=120 * 1024 * 1024),
    )(A_x.reshape(S, D), A_mem0.reshape(M, D), gate_w.reshape(1, D),
      A_Wq.reshape(D, HE), A_Wk.reshape(D, HE), A_Wv.reshape(D, HE), A_Wo.reshape(HE, D),
      B_w_gate, B_w_up, B_w_down)
    return out.reshape(1, S, D)
```
